```python
import jax
import jax.numpy as jnp

def _softmax(x, axis=-1):
    return jax.nn.softmax(x, axis=axis)
def _gelu(x):
    return jax.nn.gelu(x, approximate=True)
def _silu(x):
    return jax.nn.silu(x)
def _sigmoid(x):
    return jax.nn.sigmoid(x)
def _layernorm(x, axis=-1, eps=1e-5):
    m = jnp.mean(x, axis=axis, keepdims=True)
    v = jnp.var(x, axis=axis, keepdims=True)
    return (x - m) / jnp.sqrt(v + eps)
def _scatter_add(tgt, idx, src, axis=0):
    return tgt.at[idx].add(src)
def _segment_sum(src, seg, n):
    return jax.ops.segment_sum(src, seg, n)
class _Rng:
    def __init__(self, key):
        self._k = key
    def _next(self):
        self._k, sub = jax.random.split(self._k)
        return sub
    def normal(self, shape):
        return jax.random.normal(self._next(), shape, dtype=jnp.bfloat16)
    def randint(self, lo, hi, shape):
        return jax.random.randint(self._next(), shape, lo, hi, dtype=jnp.int32)
    def uniform(self, shape, lo=0.0, hi=1.0):
        return jax.random.uniform(self._next(), shape, jnp.bfloat16, lo, hi)
    def permutation(self, n):
        return jax.random.permutation(self._next(), n)


kernel_name = 'interleave_layers__ssm_conv_h3__mixer_s_mlp__prompt'

def setup_inputs():
    _rng = _Rng(jax.random.key(int.from_bytes(__import__("os").urandom(4), "little")))
    _w = (lambda a: (lambda t: t.astype(jnp.bfloat16) if jnp.issubdtype(t.dtype, jnp.floating) else t)(jnp.asarray(a)))
    def _A_setup():
        B, S, D = 1, 2048, 1024
        ks = 4
        return {
            "q": _w((lambda *s: _rng.normal(s) * 0.05)(B, S, D)),
            "k": _w((lambda *s: _rng.normal(s) * 0.05)(B, S, D)),
            "v": _w((lambda *s: _rng.normal(s) * 0.05)(B, S, D)),
            "shift_k": _w((lambda *s: _rng.normal(s) * 0.05)(D, ks) * 0.5),
            "ssm_k": _w((lambda *s: _rng.normal(s) * 0.05)(D, S) * (1.0 / S ** 0.5)),
            "ssm_D": _w((lambda *s: _rng.normal(s) * 0.05)(D)),
        }
    _A_in = _A_setup()

    def _B_setup():
        B, S, D, F = 1, 2048, 1024, 3584
        return {
            "x":  _w((lambda *s: _rng.normal(s) * 0.05)(B, S, D)),
            "w1": _w((lambda *s: _rng.normal(s) * 0.05)(D, D) * (D ** -0.5)),
            "w2": _w((lambda *s: _rng.normal(s) * 0.05)(D, D) * (D ** -0.5)),
            "w3": _w((lambda *s: _rng.normal(s) * 0.05)(D, F) * (D ** -0.5)),
            "w4": _w((lambda *s: _rng.normal(s) * 0.05)(F, D) * (F ** -0.5)),
        }
    _B_in = _B_setup()

    return {
        "A_q": _A_in["q"],
        "A_k": _A_in["k"],
        "A_v": _A_in["v"],
        "A_shift_k": _A_in["shift_k"],
        "A_ssm_k": _A_in["ssm_k"],
        "A_ssm_D": _A_in["ssm_D"],
        "B_x": _B_in["x"],
        "B_w1": _B_in["w1"],
        "B_w2": _B_in["w2"],
        "B_w3": _B_in["w3"],
        "B_w4": _B_in["w4"],
    }

def reference(A_q, A_k, A_v, A_shift_k, A_ssm_k, A_ssm_D, B_x, B_w1, B_w2, B_w3, B_w4):
    def _A_ref(q, k, v, shift_k, ssm_k, ssm_D):
        B, S, D = q.shape
        ks = shift_k.shape[-1]
        k_pad = jnp.pad(k, ((0, 0), (ks - 1, 0), (0, 0)))
        k_shift = jnp.zeros_like(k)
        for t in range(ks):
            k_shift = k_shift + k_pad[:, t:t + S, :] * shift_k[:, ks - 1 - t][None, None, :]
        kv = k_shift * v
        L = 2 * S
        kv_pad = jnp.pad(kv, ((0, 0), (0, S), (0, 0)))
        kf_pad = jnp.pad(ssm_k, ((0, 0), (0, S)))
        kv_f = (lambda x, axes=(-2,-1): jnp.fft.rfft2(x.astype(jnp.float32), axes=axes))(kv_pad[:, None, :, :], axes=(1, 2))
        kf_f = (lambda x, axes=(-2,-1): jnp.fft.rfft2(x.astype(jnp.float32), axes=axes))(kf_pad[:, None, :], axes=(1, 2))
        kf_f = (lambda x, *d: x.transpose(*d))(kf_f, 1, 2, 0)
        y_f = kv_f * kf_f[None, :, :, :]
        y = (lambda x, s, axes=(-2,-1): jnp.fft.irfft2(x, s=s, axes=axes).astype(jnp.bfloat16))(y_f, (1, L), axes=(1, 2))[:, 0, :S, :]
        y = y + kv * ssm_D[None, None, :]
        return q * y

    def _B_ref(x, w1, w2, w3, w4):
        B, S, D = x.shape
        h = _gelu(_layernorm(x, axis=-1) @ w1)
        c = D // 4
        g0 = jnp.pad(h[:, :, 0*c:1*c], ((0, 0), (1, 0), (0, 0)))[:, :S, :]
        g1 = jnp.pad(h[:, :, 1*c:2*c], ((0, 0), (0, 1), (0, 0)))[:, 1:, :]
        g2 = jnp.pad(h[:, :, 2*c:3*c], ((0, 0), (2, 0), (0, 0)))[:, :S, :]
        g3 = jnp.pad(h[:, :, 3*c:   ], ((0, 0), (0, 2), (0, 0)))[:, 2:, :]
        hs = jnp.concatenate([g0, g1, g2, g3], axis=-1) @ w2
        x1 = x + hs
        h2 = _gelu(_layernorm(x1, axis=-1) @ w3) @ w4
        return x1 + h2

    x = A_q
    x = x + _A_ref(_layernorm(x, axis=-1), A_k, A_v, A_shift_k, A_ssm_k, A_ssm_D)
    x = x + _B_ref(_layernorm(x, axis=-1), B_w1, B_w2, B_w3, B_w4)
    x = x + _A_ref(_layernorm(x, axis=-1), A_k, A_v, A_shift_k, A_ssm_k, A_ssm_D)
    x = x + _B_ref(_layernorm(x, axis=-1), B_w1, B_w2, B_w3, B_w4)
    return x
```

```python
import numpy as np
import jax
import jax.numpy as jnp
from jax import lax
import jax.experimental.pallas as pl
import jax.experimental.pallas.tpu as pltpu

S, D, F = 2048, 1024, 3584
KS = 4
P = 1024
N1, N2 = 16, 64
CB = 256
NCB = D // CB
TM = 256
NT = S // TM
FC = 512
PAD = 8
EPS = 1e-5
BF = jnp.bfloat16
F32 = jnp.float32


def _dft_consts():
    k1 = np.arange(N1)
    n1 = np.arange(N1)
    f1 = np.exp(-2j * np.pi * np.outer(k1 - 0.25, n1) / N1)
    f1r = np.stack([f1.real, f1.imag], axis=1)
    l1 = np.einsum("krn,st->krsnt", f1r, np.eye(8)).reshape(N1 * 16, N1 * 8)
    k2 = np.arange(N2)
    n2 = np.arange(N2)
    freq = k1[:, None, None] + N1 * k2[None, :, None] - 0.25
    m = np.exp(-2j * np.pi * freq * n2[None, None, :] / P)
    blk = np.stack([np.stack([m.real, -m.imag], axis=2),
                    np.stack([m.imag, m.real], axis=2)], axis=1)
    blk = blk.reshape(N1, 2, N2, 2, 8, 8).transpose(0, 1, 2, 4, 3, 5)
    l2 = blk.reshape(N1, 2 * N2, 2 * N2)
    l3 = l2.transpose(0, 2, 1)
    l4 = l1.T / P
    return (l1.astype(np.float32), l2.astype(np.float32),
            l3.astype(np.float32), l4.astype(np.float32))


def _ln(x):
    m = jnp.mean(x, axis=-1, keepdims=True)
    c = x - m
    v = jnp.mean(c * c, axis=-1, keepdims=True)
    return c * lax.rsqrt(v + EPS)


def _gelu(x):
    c = float(np.sqrt(2.0 / np.pi))
    return 0.5 * x * (1.0 + jnp.tanh(c * (x + 0.044715 * (x * x * x))))


def _dot(a, b):
    return jnp.dot(a, b, preferred_element_type=F32)


def _kernel(q_hbm, k_hbm, v_hbm, sk_ref, h_hbm, sd_ref, w1_hbm, w2_hbm, w3_hbm, w4_hbm,
            l1_ref, l2_ref, l3_ref, l4_ref, o_hbm,
            q_v, k_v, v_v, f_v, w1_v, w2_v, w3_v, w4_v, y_v,
            kf_s, kv_s, ft_s, a_s, b_s,
            x1_s, xn_s, ha_s, hb_s, g_s, o_s,
            sem_c, sem_w, sem_o):
    def conv_copies(c):
        cs = pl.ds(c * CB, CB)
        return (pltpu.make_async_copy(k_hbm.at[:, cs], k_v.at[c], sem_c.at[0, c]),
                pltpu.make_async_copy(v_hbm.at[:, cs], v_v.at[c], sem_c.at[1, c]),
                pltpu.make_async_copy(h_hbm.at[cs, :], f_v.at[c], sem_c.at[2, c]))

    w_copies = (pltpu.make_async_copy(q_hbm, q_v, sem_w.at[0]),
                pltpu.make_async_copy(w1_hbm, w1_v, sem_w.at[1]),
                pltpu.make_async_copy(w2_hbm, w2_v, sem_w.at[2]),
                pltpu.make_async_copy(w3_hbm, w3_v, sem_w.at[3]),
                pltpu.make_async_copy(w4_hbm, w4_v, sem_w.at[4]))
    for c in range(NCB):
        for cp in conv_copies(c):
            cp.start()
    for cp in w_copies:
        cp.start()

    zpad = jnp.zeros((PAD, D), F32)
    kf_s[0:PAD, :] = jnp.zeros((PAD, CB), F32)
    for hbuf in (ha_s, hb_s):
        hbuf[0:PAD, :] = zpad
        hbuf[PAD + S:PAD + S + PAD, :] = zpad

    def conv_block(c, carry):
        for cp in conv_copies(c):
            cp.wait()
        kf_s[PAD:PAD + S, :] = k_v[c].astype(F32)
        sk = sk_ref[c]
        RC = 256
        for r in range(S // RC):
            acc = kf_s[PAD + r * RC:PAD + (r + 1) * RC, :] * sk[0:1, :]
            for t in range(1, KS):
                acc = acc + kf_s[PAD + r * RC - t:PAD + (r + 1) * RC - t, :] * sk[t:t + 1, :]
            kv = acc * v_v[c, r * RC:(r + 1) * RC, :].astype(F32)
            kv_s[r * 4:(r + 1) * 4] = kv.reshape(4, 8, 8, CB)
        ft_s[...] = f_v[c].astype(F32).T.reshape(2 * N1, 8, 8, CB)
        l1 = l1_ref[...]
        for j in range(2):
            for g in range(8):
                for src, off in ((kv_s, 0), (ft_s, 2)):
                    rhs = src[j * N1:(j + 1) * N1, g].reshape(N1 * 8, CB).astype(BF)
                    out = _dot(l1, rhs).astype(BF)
                    a_s[:, g, :, (off + j) * CB:(off + j + 1) * CB] = out.reshape(N1, 16, CB)
        for k1 in range(N1):
            xf = _dot(l2_ref[k1], a_s[k1].reshape(2 * N2, 4 * CB))
            re, im = xf[:N2], xf[N2:]
            x0r, x1r, h0r, h1r = (re[:, i * CB:(i + 1) * CB] for i in range(4))
            x0i, x1i, h0i, h1i = (im[:, i * CB:(i + 1) * CB] for i in range(4))
            g1r = h1r + h0i
            g1i = h1i - h0r
            z0r = x0r * h0r - x0i * h0i
            z0i = x0r * h0i + x0i * h0r
            z1r = x0r * g1r - x0i * g1i + (x1r * h0r - x1i * h0i)
            z1i = x0r * g1i + x0i * g1r + (x1r * h0i + x1i * h0r)
            z = jnp.concatenate([jnp.concatenate([z0r, z1r], axis=1),
                                 jnp.concatenate([z0i, z1i], axis=1)], axis=0).astype(BF)
            b_s[:, k1] = _dot(l3_ref[k1], z).astype(BF).reshape(8, 16, 2 * CB)
        l4 = l4_ref[...]
        sd = sd_ref[c]
        for g in range(8):
            yv = _dot(l4, b_s[g].reshape(N1 * 16, 2 * CB))
            for j in range(2):
                kvg = kv_s[j * N1:(j + 1) * N1, g]
                kv_s[j * N1:(j + 1) * N1, g] = yv[:, j * CB:(j + 1) * CB].reshape(N1, 8, CB) + kvg * sd
        y_v[c] = kv_s[...].reshape(S, CB).astype(BF)
        return carry

    lax.fori_loop(0, NCB, conv_block, 0)

    def phase_a(x, r0, h_dst):
        rows = pl.ds(r0, TM)
        y = jnp.concatenate([y_v[c, rows, :] for c in range(NCB)], axis=1).astype(F32)
        x1 = x + _ln(x) * y
        xn = _ln(x1)
        x1_s[rows, :] = x1
        xn_s[rows, :] = xn
        h = _gelu(_dot(_ln(xn).astype(BF), w1_v[...]))
        h_dst[pl.ds(r0 + PAD, TM), :] = h

    def phase_b(r0, h_src):
        rows = pl.ds(r0, TM)
        c4 = D // 4
        win = h_src
        parts = []
        for gi, sh in enumerate((1, -1, 2, -2)):
            w = win[pl.ds(r0, TM + 2 * PAD), gi * c4:(gi + 1) * c4]
            parts.append(w[PAD - sh:PAD - sh + TM])
        hs = _dot(jnp.concatenate(parts, axis=1).astype(BF), w2_v[...])
        xp = xn_s[rows, :] + hs
        xb = _ln(xp).astype(BF)
        for f in range(F // FC):
            g_s[:, f * FC:(f + 1) * FC] = _gelu(_dot(xb, w3_v[:, f * FC:(f + 1) * FC])).astype(BF)
        h2 = _dot(g_s[...], w4_v[...])
        return x1_s[rows, :] + (xp + h2)

    w_copies[0].wait()
    w_copies[1].wait()

    def loop0(i, carry):
        r0 = pl.multiple_of(i * TM, TM)
        phase_a(q_v[pl.ds(r0, TM), :].astype(F32), r0, ha_s)
        return carry

    lax.fori_loop(0, NT, loop0, 0)
    for cp in w_copies[2:]:
        cp.wait()

    def loop1(i, carry):
        r0 = pl.multiple_of(i * TM, TM)
        phase_a(phase_b(r0, ha_s), r0, hb_s)
        return carry

    lax.fori_loop(0, NT, loop1, 0)

    def out_copy(i):
        r0 = pl.multiple_of(i * TM, TM)
        return pltpu.make_async_copy(o_s.at[pl.ds(r0, TM)], o_hbm.at[pl.ds(r0, TM)], sem_o.at[i])

    def loop2(i, carry):
        r0 = pl.multiple_of(i * TM, TM)
        o_s[pl.ds(r0, TM), :] = phase_b(r0, hb_s).astype(BF)
        out_copy(i).start()
        return carry

    lax.fori_loop(0, NT, loop2, 0)
    for i in range(NT):
        out_copy(i).wait()


@jax.jit
def pallas_interleave_layers__ssm_conv_h3__mixer_s_mlp__prompt_kernel(
    A_q, A_k, A_v, A_shift_k, A_ssm_k, A_ssm_D, B_x, B_w1, B_w2, B_w3, B_w4,
):
    del B_x
    l1, l2, l3, l4 = (jnp.asarray(m, dtype=BF) for m in _dft_consts())
    sk = A_shift_k.astype(F32).T.reshape(KS, NCB, CB).transpose(1, 0, 2)
    sd = A_ssm_D.astype(F32).reshape(NCB, 1, CB)
    hbm = pl.BlockSpec(memory_space=pl.ANY)
    vmem = pl.BlockSpec(memory_space=pltpu.VMEM)
    out = pl.pallas_call(
        _kernel,
        out_shape=jax.ShapeDtypeStruct((S, D), BF),
        in_specs=[hbm, hbm, hbm, vmem, hbm, vmem, hbm, hbm, hbm, hbm, vmem, vmem, vmem, vmem],
        out_specs=hbm,
        scratch_shapes=[
            pltpu.VMEM((S, D), BF),
            pltpu.VMEM((NCB, S, CB), BF),
            pltpu.VMEM((NCB, S, CB), BF),
            pltpu.VMEM((NCB, CB, S), BF),
            pltpu.VMEM((D, D), BF), pltpu.VMEM((D, D), BF),
            pltpu.VMEM((D, F), BF), pltpu.VMEM((F, D), BF),
            pltpu.VMEM((NCB, S, CB), BF),
            pltpu.VMEM((PAD + S, CB), F32),
            pltpu.VMEM((2 * N1, 8, 8, CB), F32),
            pltpu.VMEM((2 * N1, 8, 8, CB), F32),
            pltpu.VMEM((N1, 8, 16, 4 * CB), BF),
            pltpu.VMEM((8, N1, 16, 2 * CB), BF),
            pltpu.VMEM((S, D), F32), pltpu.VMEM((S, D), F32),
            pltpu.VMEM((S + 2 * PAD, D), F32), pltpu.VMEM((S + 2 * PAD, D), F32),
            pltpu.VMEM((TM, F), BF),
            pltpu.VMEM((S, D), BF),
            pltpu.SemaphoreType.DMA((3, NCB)),
            pltpu.SemaphoreType.DMA((5,)),
            pltpu.SemaphoreType.DMA((NT,)),
        ],
        compiler_params=pltpu.CompilerParams(vmem_limit_bytes=120 * 1024 * 1024),
    )(A_q.reshape(S, D), A_k.reshape(S, D), A_v.reshape(S, D), sk, A_ssm_k, sd,
      B_w1, B_w2, B_w3, B_w4, l1, l2, l3, l4)
    return out.reshape(1, S, D)
```

```python
import functools

import numpy as np
import jax
import jax.numpy as jnp
from jax import lax
import jax.experimental.pallas as pl
import jax.experimental.pallas.tpu as pltpu

S, D, F = 2048, 1024, 3584
KS = 4
P = 1024
N1, N2 = 16, 64
CB = 256
NCB = D // CB
TM = 256
NT = S // TM
HM, HD, HF = TM // 2, D // 2, F // 2
NC = 128
RG = 16
RB = 32
E1, E2 = 3, 2
LAG = 2
LEAD = 3
RING = 4
AHEAD = 3
PAD = 8
EPS = 1e-5
BF = jnp.bfloat16
F32 = jnp.float32
U32 = jnp.uint32


def _dft_consts():
    k1 = np.arange(N1)
    n1 = np.arange(N1)
    f1 = np.exp(-2j * np.pi * np.outer(k1 - 0.25, n1) / N1)
    f1r = np.stack([f1.real, f1.imag], axis=1)
    l1 = np.einsum("krn,st->krsnt", f1r, np.eye(8)).reshape(N1 * 16, N1 * 8)
    k2 = np.arange(N2)
    n2 = np.arange(N2)
    freq = k1[:, None, None] + N1 * k2[None, :, None] - 0.25
    m = np.exp(-2j * np.pi * freq * n2[None, None, :] / P)
    blk = np.stack([np.stack([m.real, -m.imag], axis=2),
                    np.stack([m.imag, m.real], axis=2)], axis=1)
    blk = blk.reshape(N1, 2, N2, 2, 8, 8).transpose(0, 1, 2, 4, 3, 5)
    l2 = blk.reshape(N1, 2 * N2, 2 * N2)
    l3 = l2.transpose(0, 2, 1)
    l4 = l1.T / P
    return (l1.astype(np.float32), l2.astype(np.float32),
            l3.astype(np.float32), l4.astype(np.float32))


def _ln(x):
    m = jnp.mean(x, axis=-1, keepdims=True)
    c = x - m
    v = jnp.mean(c * c, axis=-1, keepdims=True)
    return c * lax.rsqrt(v + EPS)


def _gelu(x):
    c = float(np.sqrt(2.0 / np.pi))
    return 0.5 * x * (1.0 + jnp.tanh(c * (x + 0.044715 * (x * x * x))))


def _dot(a, b):
    return jnp.dot(a, b, preferred_element_type=F32)


def _lhs_terms(a11, a12, a21, a22):
    return (a11 + a22, a21 + a22, a11, a22, a11 + a12, a21 - a11, a12 - a22)


def _token(col):
    t = col[:RG]
    for r in range(RG, col.shape[0], RG):
        t = t + col[r:r + RG]
    return jnp.broadcast_to(t, (RG, 128)).astype(BF)


def _after(x, order):
    if order is None or len(order) <= LEAD:
        return x
    w = min(x.shape[1], 128)
    val = jnp.broadcast_to(order[-LEAD][:1, :w].astype(F32), (x.shape[0], w))
    head = jnp.where(order[0], val, x[:, :w])
    return head if w == x.shape[1] else jnp.concatenate([head, x[:, w:]], axis=1)


def _ln_steps(x, order):
    m = jnp.mean(x, axis=-1, keepdims=True)
    yield _token(m)
    c = x - _after(m, order)
    r = lax.rsqrt(jnp.mean(c * c, axis=-1, keepdims=True) + EPS)
    yield _token(r)
    return c * _after(r, order)


def _store_lhs(dst, g, a):
    k = a.shape[1] // 2
    for i, t in enumerate(_lhs_terms(a[:RB, :k], a[:RB, k:], a[RB:, :k], a[RB:, k:])):
        t = t.astype(BF)
        dst[i, g * RB:(g + 1) * RB, :] = t
    return t[RB - RG:, k - 128:]


def _tied(a, tie):
    if tie is None or tie[0] is None:
        return a
    never, val = tie
    w = min(a.shape[1], 512)
    head = jnp.where(never, jnp.concatenate([val] * (w // 128), axis=1), a[:RG, :w])
    if w < a.shape[1]:
        head = jnp.concatenate([head, a[:RG, w:]], axis=1)
    return jnp.concatenate([head, a[RG:]], axis=0)


def _strassen(a_ref, w_ref, n, order=None):
    m = []
    for i in range(7):
        tie = yield
        a = _tied(a_ref[i], tie)
        if order is not None and len(order) > LAG:
            a = _tied(a, (order[0], order[-LAG]))
        m.append(_dot(a, w_ref.bitcast(BF)[i, :, n * NC:(n + 1) * NC]))
        if order is not None:
            order.append(m[-1][:RG, :128].astype(BF))
    m1, m2, m3, m4, m5, m6, m7 = m
    return {(0, 0): m1 + m4 - m5 + m7, (0, 1): m3 + m5,
            (1, 0): m2 + m4, (1, 1): m1 - m2 + m3 + m6}


def _chain(*gens):
    for gen in gens:
        yield from gen


def _merge(dense, sparse):
    for i, val in enumerate(dense):
        extra = next(sparse, None) if i % 2 else None
        yield val if extra is None else val + extra
    yield from sparse


def _run(main, side=(), every=1, never=None):
    side = iter(side)
    next(main)
    i = 0
    while True:
        i += 1
        val = next(side, None) if i % every == 0 and i > 1 else None
        try:
            main.send(None if val is None else (never, val))
        except StopIteration:
            break
    for _ in side:
        pass


def pairs(gen):
    for i, val in enumerate(gen):
        if i % 2:
            yield val


def _conv_phase(q_hbm, k_hbm, v_hbm, sk_ref, h_hbm, sd_ref, w1_hbm, w2_hbm, w3_hbm, w4_hbm,
                l1_ref, l2_ref, l3_ref, l4_ref, q_v, w1_v, w2_v, w3_v, w4_v, y_v,
                k_v, v_v, f_v, kf_s, kv_s, ft_s, a_s, b_s, sem_c, sem_q, sem_w):
    weights = ((w1_hbm, w1_v), (w2_hbm, w2_v), (w3_hbm, w3_v), (w4_hbm, w4_v))

    def conv_copies(c):
        cs = pl.ds(c * CB, CB)
        return (pltpu.make_async_copy(h_hbm.at[cs, :], f_v.at[c], sem_c.at[2, c]),
                pltpu.make_async_copy(k_hbm.at[:, cs], k_v.at[c], sem_c.at[0, c]),
                pltpu.make_async_copy(v_hbm.at[:, cs], v_v.at[c], sem_c.at[1, c]))

    def weight_copies(c):
        cps = []
        for i, (w_hbm, w_v) in enumerate(weights):
            k, n = w_hbm.shape[0] // 2, w_hbm.shape[1] // 2
            rows = k // NCB
            for a in range(2):
                for b in range(2):
                    cps.append(pltpu.make_async_copy(
                        w_hbm.at[pl.ds(a * k + c * rows, rows), pl.ds(b * n, n)],
                        w_v.bitcast(BF).at[1 + 2 * a + b, pl.ds(c * rows, rows)],
                        sem_w.at[c, 4 * i + 2 * a + b]))
        return cps

    def prep_weights(c):
        for _, w_v in weights:
            w_b = w_v.bitcast(BF)
            k, n = w_b.shape[1:]
            rows = k // NCB
            for r in range(0, rows, RG):
                rs = pl.ds(pl.multiple_of(c * rows + r, RG), RG)
                b11, b12, b21, b22 = (w_b[i, rs, :].astype(F32) for i in (1, 2, 3, 4))
                for i, t in ((0, b11 + b22), (2, b12 - b22), (3, b21 - b11), (5, b11 + b12), (6, b21 + b22)):
                    t = t.astype(BF)
                    w_b[i, rs, :] = t
                yield t[:, :128]

    def load_filter(c):
        for i in range(S // 128):
            t = f_v[c, :, i * 128:(i + 1) * 128].astype(F32).T
            ft_s[2 * i:2 * i + 2] = t.reshape(2, 8, 8, CB)
            yield t[:RG, :128].astype(BF)

    q_copy = pltpu.make_async_copy(q_hbm, q_v, sem_q.at[0])
    for cp in conv_copies(0):
        cp.start()
    for cp in weight_copies(0):
        cp.start()
    kf_s[0:PAD, :] = jnp.zeros((PAD, CB), F32)
    conv_copies(0)[0].wait()
    _run(load_filter(0))

    def conv_block(c, carry):
        never = c < 0

        @pl.when(c + 1 < NCB)
        def _():
            for cp in conv_copies(c + 1):
                cp.start()
            for cp in weight_copies(c + 1):
                cp.start()

        @pl.when(c + 1 == NCB)
        def _():
            q_copy.start()

        for cp in conv_copies(c)[1:]:
            cp.wait()

        def short_conv():
            kf_s[PAD:PAD + S, :] = k_v[c].astype(F32)
            sk = sk_ref[c]
            rc = 128
            for r in range(S // rc):
                acc = kf_s[PAD + r * rc:PAD + (r + 1) * rc, :] * sk[0:1, :]
                for t in range(1, KS):
                    acc = acc + kf_s[PAD + r * rc - t:PAD + (r + 1) * rc - t, :] * sk[t:t + 1, :]
                kv = acc * v_v[c, r * rc:(r + 1) * rc, :].astype(F32)
                kv_s[r * 2:(r + 1) * 2] = kv.reshape(2, 8, 8, CB)
                yield kv[:RG, :128].astype(BF)

        def stage1(src, off):
            for j in range(2):
                for g in range(8):
                    tie = yield
                    rhs = src[j * N1:(j + 1) * N1, g].reshape(N1 * 8, CB).astype(BF)
                    out = _dot(l1_ref[...], _tied(rhs, tie)).astype(BF)
                    a_s[:, g, :, (off + j) * CB:(off + j + 1) * CB] = out.reshape(N1, 16, CB)

        def stage2():
            def forward(k1, tie):
                return _dot(l2_ref[k1], _tied(a_s[k1].reshape(2 * N2, 4 * CB), tie))

            nxt = forward(0, (yield))
            for k1 in range(N1):
                xf = nxt
                if k1 + 1 < N1:
                    nxt = forward(k1 + 1, (yield))
                re, im = xf[:N2], xf[N2:]
                x0r, x1r, h0r, h1r = (re[:, i * CB:(i + 1) * CB] for i in range(4))
                x0i, x1i, h0i, h1i = (im[:, i * CB:(i + 1) * CB] for i in range(4))
                g1r = h1r + h0i
                g1i = h1i - h0r
                z0r = x0r * h0r - x0i * h0i
                z0i = x0r * h0i + x0i * h0r
                z1r = x0r * g1r - x0i * g1i + (x1r * h0r - x1i * h0i)
                z1i = x0r * g1i + x0i * g1r + (x1r * h0i + x1i * h0r)
                z = jnp.concatenate([jnp.concatenate([z0r, z1r], axis=1),
                                     jnp.concatenate([z0i, z1i], axis=1)], axis=0).astype(BF)
                tie = yield
                b_s[:, k1] = _dot(l3_ref[k1], _tied(z, tie)).astype(BF).reshape(8, 16, 2 * CB)

        def stage3():
            sd = sd_ref[c]
            for g in range(8):
                tie = yield
                yv = _dot(l4_ref[...], _tied(b_s[g].reshape(N1 * 16, 2 * CB), tie))
                for j in range(2):
                    kvg = kv_s[j * N1:(j + 1) * N1, g]
                    kv_s[j * N1:(j + 1) * N1, g] = yv[:, j * CB:(j + 1) * CB].reshape(N1, 8, CB) + kvg * sd

        _run(stage1(ft_s, 2), short_conv())
        _run(stage1(kv_s, 0))
        for cp in weight_copies(c):
            cp.wait()
        _run(stage2(), pairs(prep_weights(c)))
        nc = jnp.minimum(c + 1, NCB - 1)

        @pl.when(c + 1 < NCB)
        def _():
            conv_copies(c + 1)[0].wait()

        _run(stage3(), pairs(load_filter(nc)))
        y_v[c] = kv_s[...].reshape(NT, TM, CB).astype(BF)
        return carry

    lax.fori_loop(0, NCB, conv_block, 0)
    q_copy.wait()


def _mlp_phase(o_hbm, q_v, w1_v, w2_v, w3_v, w4_v, y_v,
               x1_s, xn_s, xp_s, res_s, x2_s, h_s, tmp_s, xa_s, xh_s, xb_s, g_s, o_s, sem_o):
    zpad = jnp.zeros((PAD, D), F32)
    for layer in range(2):
        h_s[layer, 0:PAD, :] = zpad
        h_s[layer, PAD + S:PAD + S + PAD, :] = zpad

    def both(ref, g):
        return jnp.concatenate([ref[i * HM + g * RB:i * HM + (g + 1) * RB, :] for i in range(2)], axis=0)

    def put(ref, g, val):
        for i in range(2):
            ref[i * HM + g * RB:i * HM + (g + 1) * RB, :] = val[i * RB:(i + 1) * RB]

    def gate(v, order=None):
        t, slot = v % NT, v % RING
        last = None
        for g in range(HM // RB):
            x = jnp.where(v < NT, both(q_v.at[t], g).astype(F32), both(x2_s.at[t], g))
            x = _after(x, order)
            xl = yield from _ln_steps(x, order)
            y = jnp.concatenate([both(y_v.at[c, t], g) for c in range(NCB)], axis=1).astype(F32)
            x1 = x + xl * y
            put(x1_s.at[slot], g, x1)
            xn = yield from _ln_steps(x1, order)
            put(xn_s.at[slot], g, xn)
            xa = yield from _ln_steps(xn, order)
            last = _store_lhs(xa_s.at[0], g, xa)
            yield last

    def project(v):
        r0 = pl.multiple_of((v % NT) * TM + PAD, 8)
        for n in range(HD // NC):
            cs = yield from _strassen(xa_s.at[v // (32 + n)], w1_v, n)
            for (i, j), c in cs.items():
                h_s[v // NT, pl.ds(r0 + i * HM, HM), j * HD + n * NC:j * HD + (n + 1) * NC] = _gelu(c)

    def shift(v):
        c4 = D // 4

        def fn(r):
            r0 = pl.multiple_of((v % NT) * TM + r, 8)
            parts = []
            for gi, sh in enumerate((1, -1, 2, -2)):
                w = h_s[v // NT, pl.ds(r0, RB + 2 * PAD), gi * c4:(gi + 1) * c4]
                parts.append(w[PAD - sh:PAD - sh + RB])
            return jnp.concatenate(parts, axis=1)
        for g in range(HM // RB):
            yield _store_lhs(xh_s.at[0], g, jnp.concatenate([fn(i * HM + g * RB) for i in range(2)], axis=0))

    def mix(v, order=None):
        for n in range(HD // NC):
            cs = yield from _strassen(xh_s.at[v // (32 + n)], w2_v, n, order)
            for (i, j), c in cs.items():
                rs = slice(i * HM, (i + 1) * HM)
                cols = slice(j * HD + n * NC, j * HD + (n + 1) * NC)
                xp_s[rs, cols] = xn_s[v % RING, rs, cols] + c

    def norm(v, order=None):
        last = None
        for g in range(HM // RB):
            xp = _after(both(xp_s, g), order)
            put(res_s.at[v % 2], g, xp)
            xb = yield from _ln_steps(xp, order)
            last = _store_lhs(xb_s.at[0], g, xb)
            yield last

    def up(u, order):
        for n in range(HF // NC):
            cs = yield from _strassen(xb_s.at[u // (32 + n)], w3_v, n, order)
            g = {ij: _gelu(c) for ij, c in cs.items()}
            for i, t in enumerate(_lhs_terms(g[0, 0], g[0, 1], g[1, 0], g[1, 1])):
                g_s[0, i, :, n * NC:(n + 1) * NC] = t.astype(BF)

    def down(u, order):
        for n in range(HD // NC):
            cs = yield from _strassen(g_s.at[u // (32 + n)], w4_v, n, order)
            for (i, j), c in cs.items():
                rs = slice(i * HM, (i + 1) * HM)
                cols = slice(j * HD + n * NC, j * HD + (n + 1) * NC)
                x2 = x1_s[u % RING, rs, cols] + (res_s[u % 2, rs, cols] + c)
                x2_s[u % NT, rs, cols] = x2
                o_s[u % NT, rs, cols] = x2.astype(BF)

    def out_copy(i):
        return pltpu.make_async_copy(o_s.at[i], o_hbm.at[i], sem_o.at[i])

    def prologue(v, carry):
        _run(gate(v))
        _run(project(v))
        return carry

    lax.fori_loop(0, AHEAD, prologue, 0)
    _run(_chain(shift(0), mix(0), norm(0)))

    def main(u, carry):
        nxt = jnp.minimum(u + 1, 2 * NT - 1)
        never = u < 0
        order = [never]
        _run(up(u, order), shift(nxt), every=20, never=never)
        _run(mix(nxt, order))
        _run(down(u, order), _merge(gate(u + AHEAD, order), norm(nxt, order)), every=1, never=never)

        @pl.when(u + AHEAD < 2 * NT)
        def _():
            _run(project(u + AHEAD))

        @pl.when(u >= NT)
        def _():
            out_copy(u - NT).start()

        return carry

    lax.fori_loop(0, 2 * NT, main, 0)
    for i in range(NT):
        out_copy(i).wait()


def _kernel(*refs):
    ins, o_hbm, shared = refs[:14], refs[14], refs[15:]
    pl.run_scoped(
        functools.partial(_conv_phase, *ins, *shared),
        pltpu.VMEM((NCB, S, CB), BF),
        pltpu.VMEM((NCB, S, CB), BF),
        pltpu.VMEM((NCB, CB, S), BF),
        pltpu.VMEM((PAD + S, CB), F32),
        pltpu.VMEM((2 * N1, 8, 8, CB), F32),
        pltpu.VMEM((2 * N1, 8, 8, CB), F32),
        pltpu.VMEM((N1, 8, 16, 4 * CB), BF),
        pltpu.VMEM((8, N1, 16, 2 * CB), BF),
        pltpu.SemaphoreType.DMA((3, NCB)),
        pltpu.SemaphoreType.DMA((1,)),
        pltpu.SemaphoreType.DMA((NCB, 16)),
    )
    lhs = pltpu.VMEM((1, 7, HM, HD), BF)
    pl.run_scoped(
        functools.partial(_mlp_phase, o_hbm, *shared),
        pltpu.VMEM((RING, TM, D), F32), pltpu.VMEM((RING, TM, D), F32), pltpu.VMEM((TM, D), F32),
        pltpu.VMEM((2, TM, D), F32), pltpu.VMEM((NT, TM, D), F32),
        pltpu.VMEM((2, S + 2 * PAD, D), F32),
        pltpu.VMEM((3, 2, RG, D), F32),
        lhs, lhs, lhs,
        pltpu.VMEM((1, 7, HM, HF), BF),
        pltpu.VMEM((NT, TM, D), BF),
        pltpu.SemaphoreType.DMA((NT,)),
    )


@jax.jit
def pallas_interleave_layers__ssm_conv_h3__mixer_s_mlp__prompt_kernel(
    A_q, A_k, A_v, A_shift_k, A_ssm_k, A_ssm_D, B_x, B_w1, B_w2, B_w3, B_w4,
):
    del B_x
    l1, l2, l3, l4 = (jnp.asarray(m, dtype=BF) for m in _dft_consts())
    sk = A_shift_k.astype(F32).T.reshape(KS, NCB, CB).transpose(1, 0, 2)
    sd = A_ssm_D.astype(F32).reshape(NCB, 1, CB)
    hbm = pl.BlockSpec(memory_space=pl.ANY)
    vmem = pl.BlockSpec(memory_space=pltpu.VMEM)
    out = pl.pallas_call(
        _kernel,
        out_shape=jax.ShapeDtypeStruct((NT, TM, D), BF),
        in_specs=[hbm, hbm, hbm, vmem, hbm, vmem, hbm, hbm, hbm, hbm, vmem, vmem, vmem, vmem],
        out_specs=hbm,
        scratch_shapes=[
            pltpu.VMEM((NT, TM, D), BF),
            pltpu.VMEM((7, HD // 2, HD), U32), pltpu.VMEM((7, HD // 2, HD), U32),
            pltpu.VMEM((7, HD // 2, HF), U32), pltpu.VMEM((7, HF // 2, HD), U32),
            pltpu.VMEM((NCB, NT, TM, CB), BF),
        ],
        compiler_params=pltpu.CompilerParams(vmem_limit_bytes=120 * 1024 * 1024),
    )(A_q.reshape(NT, TM, D), A_k.reshape(S, D), A_v.reshape(S, D), sk, A_ssm_k, sd,
      B_w1, B_w2, B_w3, B_w4, l1, l2, l3, l4)
    return out.reshape(1, S, D)
```

```python
import functools

import numpy as np
import jax
import jax.numpy as jnp
from jax import lax
import jax.experimental.pallas as pl
import jax.experimental.pallas.tpu as pltpu

S, D, F = 2048, 1024, 3584
KS = 4
P = 1024
N1, N2 = 16, 64
CB = 256
NCB = D // CB
TM = 256
NT = S // TM
HM, HD, HF = TM // 2, D // 2, F // 2
NC = 128
RG = 16
RB = 32
LAG = 2
LEAD = 3
WC = 512
SLOT = ((0, 0), (1, 0), (0, 1), (0, 2), (1, 1), (0, 3), (0, 4))
W_HALVES = ((HD, HD), (HD, HD), (HD, HF), (HF, HD))
RING = 4
AHEAD = 3
PAD = 8
EPS = 1e-5
BF = jnp.bfloat16
F32 = jnp.float32
U32 = jnp.uint32


def _dft_consts():
    k1 = np.arange(N1)
    n1 = np.arange(N1)
    f1 = np.exp(-2j * np.pi * np.outer(k1 - 0.25, n1) / N1)
    f1r = np.stack([f1.real, f1.imag], axis=1)
    l1 = np.einsum("krn,st->krsnt", f1r, np.eye(8)).reshape(N1 * 16, N1 * 8)
    k2 = np.arange(N2)
    n2 = np.arange(N2)
    freq = k1[:, None, None] + N1 * k2[None, :, None] - 0.25
    m = np.exp(-2j * np.pi * freq * n2[None, None, :] / P)
    blk = np.stack([np.stack([m.real, -m.imag], axis=2),
                    np.stack([m.imag, m.real], axis=2)], axis=1)
    blk = blk.reshape(N1, 2, 8, 8, 2, 8, 8)
    l2 = blk.transpose(0, 2, 1, 3, 5, 6, 4).reshape(N1, 2 * N2, 2 * N2)
    l3 = blk.transpose(0, 5, 4, 6, 2, 3, 1).reshape(N1, 2 * N2, 2 * N2)
    l4 = l1.reshape(N1, 2, 8, N1 * 8).transpose(3, 0, 2, 1).reshape(N1 * 8, N1 * 16) / P
    return (l1.astype(np.float32), l2.astype(np.float32),
            l3.astype(np.float32), l4.astype(np.float32))


def _ln(x):
    m = jnp.mean(x, axis=-1, keepdims=True)
    c = x - m
    v = jnp.mean(c * c, axis=-1, keepdims=True)
    return c * lax.rsqrt(v + EPS)


def _gelu(x):
    c = float(np.sqrt(2.0 / np.pi))
    return 0.5 * x * (1.0 + jnp.tanh(c * (x + 0.044715 * (x * x * x))))


def _dot(a, b):
    return jnp.dot(a, b, preferred_element_type=F32)


def _pack(re, im):
    return pltpu.pack_elementwise([re, im], packed_dtype=BF).astype(U32)


def _pack_groups(x):
    x = x.reshape(x.shape[0] // 16, 2, 8, x.shape[1])
    return _pack(x[:, 0], x[:, 1])


def _lhs_terms(a11, a12, a21, a22):
    return (a11 + a22, a21 + a22, a11, a22, a11 + a12, a21 - a11, a12 - a22)


def _token(col):
    t = col[:RG]
    for r in range(RG, col.shape[0], RG):
        t = t + col[r:r + RG]
    return jnp.broadcast_to(t, (RG, 128)).astype(BF)


def _after(x, order):
    if order is None or len(order) <= LEAD:
        return x
    w = min(x.shape[1], 128)
    val = jnp.broadcast_to(order[-LEAD][:1, :w].astype(F32), (x.shape[0], w))
    head = jnp.where(order[0], val, x[:, :w])
    return head if w == x.shape[1] else jnp.concatenate([head, x[:, w:]], axis=1)


def _ln_steps(x, order):
    m = jnp.mean(x, axis=-1, keepdims=True)
    yield _token(m)
    c = x - _after(m, order)
    r = lax.rsqrt(jnp.mean(c * c, axis=-1, keepdims=True) + EPS)
    yield _token(r)
    return c * _after(r, order)


def _store_lhs(dst, g, a):
    k = a.shape[1] // 2
    for i, t in enumerate(_lhs_terms(a[:RB, :k], a[:RB, k:], a[RB:, :k], a[RB:, k:])):
        t = t.astype(BF)
        dst[i, g * RB:(g + 1) * RB, :] = t
    return t[RB - RG:, k - 128:]


def _tied(a, tie):
    if tie is None or tie[0] is None:
        return a
    never, val = tie
    w = min(a.shape[1], 512)
    head = jnp.where(never, jnp.concatenate([val] * (w // 128), axis=1), a[:RG, :w])
    if w < a.shape[1]:
        head = jnp.concatenate([head, a[:RG, w:]], axis=1)
    return jnp.concatenate([head, a[RG:]], axis=0)


def _strassen(a_ref, w_ref, n, order=None):
    m = []
    for i in range(7):
        tie = yield
        a = _tied(a_ref[i], tie)
        if order is not None and len(order) > LAG:
            a = _tied(a, (order[0], order[-LAG]))
        m.append(_dot(a, w_ref[SLOT[i][0]].bitcast(BF)[SLOT[i][1], :, n * NC:(n + 1) * NC]))
        if order is not None:
            order.append(m[-1][:RG, :128].astype(BF))
    m1, m2, m3, m4, m5, m6, m7 = m
    return {(0, 0): m1 + m4 - m5 + m7, (0, 1): m3 + m5,
            (1, 0): m2 + m4, (1, 1): m1 - m2 + m3 + m6}


def _chain(*gens):
    for gen in gens:
        yield from gen


def _merge(dense, sparse):
    for i, val in enumerate(dense):
        extra = next(sparse, None) if i % 2 else None
        yield val if extra is None else val + extra
    yield from sparse


def _run(main, side=(), every=1, never=None):
    side = iter(side)
    next(main)
    i = 0
    while True:
        i += 1
        val = next(side, None) if i % every == 0 and i > 1 else None
        try:
            main.send(None if val is None else (never, val))
        except StopIteration:
            break
    for _ in side:
        pass


def pairs(gen):
    for i, val in enumerate(gen):
        if i % 2:
            yield val


def _conv_phase(q_hbm, k_hbm, v_hbm, sk_ref, h_hbm, sd_ref, w1_hbm, w2_hbm, w3_hbm, w4_hbm,
                l1_ref, l2_ref, l3_ref, l4_ref, q_v, w1_v, w2_v, w3_v, w4_v, y_v,
                k_v, v_v, f_v, kf_s, kv_s, ft_s, a_s, b_s, s1, s2, s3, s4, sem_c, sem_q, sem_w):
    weights = ((w1_hbm, w1_v), (w2_hbm, w2_v), (w3_hbm, w3_v), (w4_hbm, w4_v))

    stage = (s1, s2, s3, s4)

    def filter_copy(c):
        return pltpu.make_async_copy(h_hbm.at[pl.ds(c * CB, CB), :], f_v.at[c], sem_c.at[2, c])

    def kv_copies(c):
        cs = pl.ds(c * CB, CB)
        return (pltpu.make_async_copy(k_hbm.at[:, cs], k_v.at[c], sem_c.at[0, c]),
                pltpu.make_async_copy(v_hbm.at[:, cs], v_v.at[c], sem_c.at[1, c]))

    def weight_copies(c):
        cps = []
        for i, (w_hbm, w_v) in enumerate(weights):
            k, n = w_hbm.shape[0] // 2, w_hbm.shape[1] // 2
            rows = k // NCB
            for a in range(2):
                for b in range(2):
                    cps.append(pltpu.make_async_copy(
                        w_hbm.at[pl.ds(a * k + c * rows, rows), pl.ds(b * n, n)],
                        w_v[1].bitcast(BF).at[a, pl.ds(c * rows, rows)] if a == b
                        else stage[i].bitcast(BF).at[c % 2, a],
                        sem_w.at[c, 4 * i + 2 * a + b]))
        return cps

    def prep_weights(c):
        for (_, w_v), st in zip(weights, stage):
            rows, n = st.shape[2:]
            for r in range(0, rows, 8):
                rs = pl.ds(pl.multiple_of(c * rows + r, 8), 8)
                for col in range(0, n, WC):
                    cs = slice(col, min(col + WC, n))
                    raw = (w_v[1][0, rs, cs], st[c % 2, 0, r:r + 8, cs], st[c % 2, 1, r:r + 8, cs], w_v[1][1, rs, cs])
                    halves = []
                    for part in range(2):
                        b11, b12, b21, b22 = (
                            pltpu.unpack_elementwise(t, index=part, packed_dtype=BF, unpacked_dtype=F32)
                            for t in raw)
                        halves.append((b11 + b22, b12 - b22, b21 - b11, b11 + b12, b21 + b22))
                    for i, (lo, hi) in enumerate(zip(*halves)):
                        w_v[0][i, rs, cs] = pltpu.pack_elementwise([lo, hi], packed_dtype=BF).astype(U32)
                yield jnp.concatenate([lo[:, -128:], hi[:, -128:]], axis=0).astype(BF)

    def load_filter(c):
        for i in range(S // 128):
            t = f_v[c, :, i * 128:(i + 1) * 128].astype(F32).T
            ft_s[2 * i:2 * i + 2] = t.reshape(2, 8, 8, CB)
            yield t[:RG, :128].astype(BF)

    q_copy = pltpu.make_async_copy(q_hbm, q_v, sem_q.at[0])
    for cp in (filter_copy(0), *kv_copies(0)):
        cp.start()
    for cp in weight_copies(0):
        cp.start()
    kf_s[0:PAD, :] = jnp.zeros((PAD, CB), F32)
    filter_copy(0).wait()
    _run(load_filter(0))

    def conv_block(c, carry):

        @pl.when(c + 1 < NCB)
        def _():
            for cp in (filter_copy(c + 1), *kv_copies(c + 1)):
                cp.start()
            for cp in weight_copies(c + 1):
                cp.start()

        @pl.when(c + 1 == NCB)
        def _():
            q_copy.start()

        for cp in kv_copies(c):
            cp.wait()

        def short_conv():
            kf_s[PAD:PAD + S, :] = k_v[c].astype(F32)
            sk = sk_ref[c]
            rc = 128
            for r in range(S // rc):
                k0 = kf_s[r * rc:PAD + (r + 1) * rc, :]
                k1 = pltpu.roll(k0, 1, 0)
                near = k0 * sk[0:1, :] + k1 * sk[1:2, :]
                far = k0 * sk[2:3, :] + k1 * sk[3:4, :]
                ks = near[PAD:] + far[PAD - 2:PAD - 2 + rc]
                kv = ks * v_v[c, r * rc:(r + 1) * rc, :].astype(F32)
                kv_s[r * 2:(r + 1) * 2] = kv.reshape(2, 8, 8, CB)
                yield kv[:RG, :128].astype(BF)

        def stage1(src, off):
            for j in range(2):
                for g in range(8):
                    tie = yield
                    rhs = src[j * N1:(j + 1) * N1, g].reshape(N1 * 8, CB).astype(BF)
                    out = _pack_groups(_dot(l1_ref[...], _tied(rhs, tie)))
                    for h in range(CB // 128):
                        col = (4 * h + off + j) * 128
                        a_s[:, 8 * g:8 * g + 8, col:col + 128] = out[:, :, h * 128:(h + 1) * 128]

        def stage2():
            def forward(k1, tie):
                out = _dot(l2_ref[k1], _tied(a_s.bitcast(BF)[k1], tie))
                return out

            nxt = forward(0, (yield))
            for k1 in range(N1):
                xf = nxt
                if k1 + 1 < N1:
                    nxt = forward(k1 + 1, (yield))
                xf = xf.reshape(8, 2, 8, 4 * CB)
                zs = []
                for h in range(CB // 128):
                    x0r, x1r, h0r, h1r = (xf[:, 0, :, (4 * h + i) * 128:(4 * h + i + 1) * 128] for i in range(4))
                    x0i, x1i, h0i, h1i = (xf[:, 1, :, (4 * h + i) * 128:(4 * h + i + 1) * 128] for i in range(4))
                    g1r = h1r + h0i
                    g1i = h1i - h0r
                    z0r = x0r * h0r - x0i * h0i
                    z0i = x0r * h0i + x0i * h0r
                    z1r = x0r * g1r - x0i * g1i + (x1r * h0r - x1i * h0i)
                    z1i = x0r * g1i + x0i * g1r + (x1r * h0i + x1i * h0r)
                    zs += [_pack(z0r, z0i), _pack(z1r, z1i)]
                z = pltpu.bitcast(jnp.concatenate(zs, axis=-1).reshape(N2, 2 * CB), BF)
                tie = yield
                b_s[:, 8 * k1:8 * k1 + 8] = _pack_groups(_dot(l3_ref[k1], _tied(z, tie)))

        def stage3():
            sd = sd_ref[c]
            for g in range(8):
                tie = yield
                yv = _dot(l4_ref[...], _tied(b_s.bitcast(BF)[g], tie))
                for j in range(2):
                    yj = jnp.concatenate(
                        [yv[:, (2 * h + j) * 128:(2 * h + j + 1) * 128] for h in range(CB // 128)], axis=1)
                    kvg = kv_s[j * N1:(j + 1) * N1, g]
                    kv_s[j * N1:(j + 1) * N1, g] = yj.reshape(N1, 8, CB) + kvg * sd

        _run(stage1(ft_s, 2), short_conv())
        _run(stage1(kv_s, 0))
        for cp in weight_copies(c):
            cp.wait()
        _run(stage2(), pairs(prep_weights(c)))
        nc = jnp.minimum(c + 1, NCB - 1)

        @pl.when(c + 1 < NCB)
        def _():
            filter_copy(c + 1).wait()

        _run(stage3(), pairs(load_filter(nc)))
        y_v[c] = kv_s[...].reshape(NT, TM, CB).astype(BF)
        return carry

    lax.fori_loop(0, NCB, conv_block, 0)
    q_copy.wait()


def _mlp_phase(o_hbm, q_v, w1_v, w2_v, w3_v, w4_v, y_v,
               x1_s, xn_s, xp_s, res_s, x2_s, h_s, xa_s, xh_s, xb_s, g_s, o_s, sem_o):
    zpad = jnp.zeros((PAD, D), F32)
    for layer in range(2):
        h_s[layer, 0:PAD, :] = zpad
        h_s[layer, PAD + S:PAD + S + PAD, :] = zpad

    def both(ref, g):
        return jnp.concatenate([ref[i * HM + g * RB:i * HM + (g + 1) * RB, :] for i in range(2)], axis=0)

    def put(ref, g, val):
        for i in range(2):
            ref[i * HM + g * RB:i * HM + (g + 1) * RB, :] = val[i * RB:(i + 1) * RB]

    def gate(v, order=None):
        t, slot = v % NT, v % RING
        last = None
        for g in range(HM // RB):
            x = jnp.where(v < NT, both(q_v.at[t], g).astype(F32), both(x2_s.at[t], g))
            x = _after(x, order)
            xl = yield from _ln_steps(x, order)
            y = jnp.concatenate([both(y_v.at[c, t], g) for c in range(NCB)], axis=1).astype(F32)
            x1 = x + xl * y
            put(x1_s.at[slot], g, x1)
            xn = yield from _ln_steps(x1, order)
            put(xn_s.at[slot], g, xn)
            xa = yield from _ln_steps(xn, order)
            last = _store_lhs(xa_s.at[0], g, xa)
            yield last

    def project(v):
        r0 = pl.multiple_of((v % NT) * TM + PAD, 8)
        for n in range(HD // NC):
            cs = yield from _strassen(xa_s.at[v // (32 + n)], w1_v, n)
            for (i, j), c in cs.items():
                h_s[v // NT, pl.ds(r0 + i * HM, HM), j * HD + n * NC:j * HD + (n + 1) * NC] = _gelu(c)

    def shift(v):
        c4 = D // 4

        def fn(r):
            r0 = pl.multiple_of((v % NT) * TM + r, 8)
            parts = []
            for gi, sh in enumerate((1, -1, 2, -2)):
                w = h_s[v // NT, pl.ds(r0, RB + 2 * PAD), gi * c4:(gi + 1) * c4]
                parts.append(w[PAD - sh:PAD - sh + RB])
            return jnp.concatenate(parts, axis=1)
        for g in range(HM // RB):
            yield _store_lhs(xh_s.at[0], g, jnp.concatenate([fn(i * HM + g * RB) for i in range(2)], axis=0))

    def mix(v, order=None):
        for n in range(HD // NC):
            cs = yield from _strassen(xh_s.at[v // (32 + n)], w2_v, n, order)
            for (i, j), c in cs.items():
                rs = slice(i * HM, (i + 1) * HM)
                cols = slice(j * HD + n * NC, j * HD + (n + 1) * NC)
                xp_s[rs, cols] = xn_s[v % RING, rs, cols] + c

    def norm(v, order=None):
        last = None
        for g in range(HM // RB):
            xp = _after(both(xp_s, g), order)
            put(res_s.at[v % 2], g, xp)
            xb = yield from _ln_steps(xp, order)
            last = _store_lhs(xb_s.at[0], g, xb)
            yield last

    def up(u, order):
        for n in range(HF // NC):
            cs = yield from _strassen(xb_s.at[u // (32 + n)], w3_v, n, order)
            g = {ij: _gelu(c) for ij, c in cs.items()}
            for i, t in enumerate(_lhs_terms(g[0, 0], g[0, 1], g[1, 0], g[1, 1])):
                g_s[0, i, :, n * NC:(n + 1) * NC] = t.astype(BF)

    def down(u, order):
        for n in range(HD // NC):
            cs = yield from _strassen(g_s.at[u // (32 + n)], w4_v, n, order)
            for (i, j), c in cs.items():
                rs = slice(i * HM, (i + 1) * HM)
                cols = slice(j * HD + n * NC, j * HD + (n + 1) * NC)
                x2 = x1_s[u % RING, rs, cols] + (res_s[u % 2, rs, cols] + c)
                x2_s[u % NT, rs, cols] = x2
                o_s[u % NT, rs, cols] = x2.astype(BF)

    def out_copy(i):
        return pltpu.make_async_copy(o_s.at[i], o_hbm.at[i], sem_o.at[i])

    def prologue(v, carry):
        _run(gate(v))
        _run(project(v))
        return carry

    lax.fori_loop(0, AHEAD, prologue, 0)
    _run(_chain(shift(0), mix(0), norm(0)))

    def main(u, carry):
        nxt = jnp.minimum(u + 1, 2 * NT - 1)
        never = u < 0
        order = [never]
        _run(up(u, order), shift(nxt), every=20, never=never)
        _run(mix(nxt, order))
        _run(down(u, order), _merge(gate(u + AHEAD, order), norm(nxt, order)), every=1, never=never)

        @pl.when(u + AHEAD < 2 * NT)
        def _():
            _run(project(u + AHEAD))

        @pl.when(u >= NT)
        def _():
            out_copy(u - NT).start()

        return carry

    lax.fori_loop(0, 2 * NT, main, 0)
    for i in range(NT):
        out_copy(i).wait()


def _kernel(*refs):
    ins, o_hbm, shared = refs[:14], refs[14], refs[15:]
    pl.run_scoped(
        functools.partial(_conv_phase, *ins, *shared),
        pltpu.VMEM((NCB, S, CB), BF),
        pltpu.VMEM((NCB, S, CB), BF),
        pltpu.VMEM((NCB, CB, S), BF),
        pltpu.VMEM((PAD + S, CB), F32),
        pltpu.VMEM((2 * N1, 8, 8, CB), F32),
        pltpu.VMEM((2 * N1, 8, 8, CB), F32),
        pltpu.VMEM((N1, N2, 4 * CB), U32),
        pltpu.VMEM((8, N1 * 8, 2 * CB), U32),
        *(pltpu.VMEM((2, 2, k // 2 // NCB, n), U32) for k, n in W_HALVES),
        pltpu.SemaphoreType.DMA((3, NCB)),
        pltpu.SemaphoreType.DMA((1,)),
        pltpu.SemaphoreType.DMA((NCB, 16)),
    )
    lhs = pltpu.VMEM((1, 7, HM, HD), BF)
    pl.run_scoped(
        functools.partial(_mlp_phase, o_hbm, *shared),
        pltpu.VMEM((RING, TM, D), F32), pltpu.VMEM((RING, TM, D), F32), pltpu.VMEM((TM, D), F32),
        pltpu.VMEM((2, TM, D), F32), pltpu.VMEM((NT, TM, D), F32),
        pltpu.VMEM((2, S + 2 * PAD, D), F32),
        lhs, lhs, lhs,
        pltpu.VMEM((1, 7, HM, HF), BF),
        pltpu.VMEM((NT, TM, D), BF),
        pltpu.SemaphoreType.DMA((NT,)),
    )


@jax.jit
def pallas_interleave_layers__ssm_conv_h3__mixer_s_mlp__prompt_kernel(
    A_q, A_k, A_v, A_shift_k, A_ssm_k, A_ssm_D, B_x, B_w1, B_w2, B_w3, B_w4,
):
    del B_x
    l1, l2, l3, l4 = (jnp.asarray(m, dtype=BF) for m in _dft_consts())
    sk = A_shift_k.astype(F32).T.reshape(KS, NCB, CB).transpose(1, 0, 2)
    sd = A_ssm_D.astype(F32).reshape(NCB, 1, CB)
    hbm = pl.BlockSpec(memory_space=pl.ANY)
    vmem = pl.BlockSpec(memory_space=pltpu.VMEM)
    out = pl.pallas_call(
        _kernel,
        out_shape=jax.ShapeDtypeStruct((NT, TM, D), BF),
        in_specs=[hbm, hbm, hbm, vmem, hbm, vmem, hbm, hbm, hbm, hbm, vmem, vmem, vmem, vmem],
        out_specs=hbm,
        scratch_shapes=[
            pltpu.VMEM((NT, TM, D), BF),
            *([pltpu.VMEM((5, k // 2, n), U32), pltpu.VMEM((2, k // 2, n), U32)] for k, n in W_HALVES),
            pltpu.VMEM((NCB, NT, TM, CB), BF),
        ],
        compiler_params=pltpu.CompilerParams(vmem_limit_bytes=120 * 1024 * 1024),
    )(A_q.reshape(NT, TM, D), A_k.reshape(S, D), A_v.reshape(S, D), sk, A_ssm_k, sd,
      B_w1, B_w2, B_w3, B_w4, l1, l2, l3, l4)
    return out.reshape(1, S, D)
```

```python
import functools

import numpy as np
import jax
import jax.numpy as jnp
from jax import lax
import jax.experimental.pallas as pl
import jax.experimental.pallas.tpu as pltpu

S, D, F = 2048, 1024, 3584
KS = 4
P = 1024
N1, N2 = 16, 64
CB = 256
NCB = D // CB
TM = 256
NT = S // TM
HM, HD, HF = TM // 2, D // 2, F // 2
NC = 128
RG = 16
RB = 32
LAG = 2
LEAD = 3
WC = 512
SLOT = ((0, 0), (1, 0), (0, 1), (0, 2), (1, 1), (0, 3), (0, 4))
W_HALVES = ((HD, HD), (HD, HD), (HD, HF), (HF, HD))
RING = 4
AHEAD = 3
PAD = 8
EPS = 1e-5
BF = jnp.bfloat16
F32 = jnp.float32
U32 = jnp.uint32


def _dft_consts():
    k1 = np.arange(N1)
    n1 = np.arange(N1)
    f1 = np.exp(-2j * np.pi * np.outer(k1 - 0.25, n1) / N1)
    f1r = np.stack([f1.real, f1.imag], axis=1)
    l1 = np.einsum("krn,st->krsnt", f1r, np.eye(8)).reshape(N1 * 16, N1 * 8)
    k2 = np.arange(N2)
    n2 = np.arange(N2)
    freq = k1[:, None, None] + N1 * k2[None, :, None] - 0.25
    m = np.exp(-2j * np.pi * freq * n2[None, None, :] / P)
    blk = np.stack([np.stack([m.real, -m.imag], axis=2),
                    np.stack([m.imag, m.real], axis=2)], axis=1)
    blk = blk.reshape(N1, 2, 8, 8, 2, 8, 8)
    l2 = blk.transpose(0, 2, 1, 3, 5, 6, 4).reshape(N1, 2 * N2, 2 * N2)
    l3 = blk.transpose(0, 5, 4, 6, 2, 3, 1).reshape(N1, 2 * N2, 2 * N2)
    l4 = l1.reshape(N1, 2, 8, N1 * 8).transpose(3, 0, 2, 1).reshape(N1 * 8, N1 * 16) / P
    return (l1.astype(np.float32), l2.astype(np.float32),
            l3.astype(np.float32), l4.astype(np.float32))


def _ln(x):
    m = jnp.mean(x, axis=-1, keepdims=True)
    c = x - m
    v = jnp.mean(c * c, axis=-1, keepdims=True)
    return c * lax.rsqrt(v + EPS)


def _gelu(x):
    c = float(np.sqrt(2.0 / np.pi))
    return 0.5 * x * (1.0 + jnp.tanh(c * (x + 0.044715 * (x * x * x))))


def _dot(a, b):
    return jnp.dot(a, b, preferred_element_type=F32)


def _pack(re, im):
    return pltpu.pack_elementwise([re, im], packed_dtype=BF).astype(U32)


def _pack_groups(x):
    x = x.reshape(x.shape[0] // 16, 2, 8, x.shape[1])
    return _pack(x[:, 0], x[:, 1])


def _lhs_terms(a11, a12, a21, a22):
    return (a11 + a22, a21 + a22, a11, a22, a11 + a12, a21 - a11, a12 - a22)


def _token(col):
    t = col[:RG]
    for r in range(RG, col.shape[0], RG):
        t = t + col[r:r + RG]
    return jnp.broadcast_to(t, (RG, 128)).astype(BF)


def _after(x, order):
    if order is None or len(order) <= LEAD:
        return x
    w = min(x.shape[1], 128)
    val = jnp.broadcast_to(order[-LEAD][:1, :w].astype(F32), (x.shape[0], w))
    head = jnp.where(order[0], val, x[:, :w])
    return head if w == x.shape[1] else jnp.concatenate([head, x[:, w:]], axis=1)


def _ln_steps(x, order):
    m = jnp.mean(x, axis=-1, keepdims=True)
    yield _token(m)
    c = x - _after(m, order)
    r = lax.rsqrt(jnp.mean(c * c, axis=-1, keepdims=True) + EPS)
    yield _token(r)
    return c * _after(r, order)


def _store_lhs(dst, g, a):
    k = a.shape[1] // 2
    for i, t in enumerate(_lhs_terms(a[:RB, :k], a[:RB, k:], a[RB:, :k], a[RB:, k:])):
        t = t.astype(BF)
        dst[i, g * RB:(g + 1) * RB, :] = t
    return t[RB - RG:, k - 128:]


def _tied(a, tie):
    if tie is None or tie[0] is None:
        return a
    never, val = tie
    w = min(a.shape[1], 512)
    head = jnp.where(never, jnp.concatenate([val] * (w // 128), axis=1), a[:RG, :w])
    if w < a.shape[1]:
        head = jnp.concatenate([head, a[:RG, w:]], axis=1)
    return jnp.concatenate([head, a[RG:]], axis=0)


def _strassen(a_ref, w_ref, n, order=None):
    m = []
    for i in range(7):
        tie = yield
        a = _tied(a_ref[i], tie)
        if order is not None and len(order) > LAG:
            a = _tied(a, (order[0], order[-LAG]))
        m.append(_dot(a, w_ref[SLOT[i][0]].bitcast(BF)[SLOT[i][1], :, n * NC:(n + 1) * NC]))
        if order is not None:
            order.append(m[-1][:RG, :128].astype(BF))
    m1, m2, m3, m4, m5, m6, m7 = m
    return {(0, 0): m1 + m4 - m5 + m7, (0, 1): m3 + m5,
            (1, 0): m2 + m4, (1, 1): m1 - m2 + m3 + m6}


def _chain(*gens):
    for gen in gens:
        yield from gen


def _merge(dense, sparse):
    for i, val in enumerate(dense):
        extra = next(sparse, None) if i % 2 else None
        yield val if extra is None else val + extra
    yield from sparse


def _run(main, side=(), every=1, never=None):
    side = iter(side)
    next(main)
    i = 0
    while True:
        i += 1
        val = next(side, None) if i % every == 0 and i > 1 else None
        try:
            main.send(None if val is None else (never, val))
        except StopIteration:
            break
    for _ in side:
        pass


def pairs(gen):
    for i, val in enumerate(gen):
        if i % 2:
            yield val


def _weight_copies(w_hbm, w_v, st, c, sems):
    k, n = w_hbm.shape[0] // 2, w_hbm.shape[1] // 2
    rows = 2 * st.shape[1]
    return [pltpu.make_async_copy(
        w_hbm.at[pl.ds(a * k + c * rows, rows), pl.ds(b * n, n)],
        w_v[1].bitcast(BF).at[a, pl.ds(c * rows, rows)] if a == b else st.bitcast(BF).at[a],
        sems.at[2 * a + b]) for a in range(2) for b in range(2)]


def _prep_weight(w_v, st, c):
    rows, n = st.shape[1:]
    for r in range(0, rows, 8):
        rs = pl.ds(pl.multiple_of(c * rows + r, 8), 8)
        for col in range(0, n, WC):
            cs = slice(col, min(col + WC, n))
            raw = (w_v[1][0, rs, cs], st[0, r:r + 8, cs], st[1, r:r + 8, cs], w_v[1][1, rs, cs])
            halves = []
            for part in range(2):
                b11, b12, b21, b22 = (
                    pltpu.unpack_elementwise(t, index=part, packed_dtype=BF, unpacked_dtype=F32)
                    for t in raw)
                halves.append((b11 + b22, b12 - b22, b21 - b11, b11 + b12, b21 + b22))
            for i, (lo, hi) in enumerate(zip(*halves)):
                w_v[0][i, rs, cs] = _pack(lo, hi)
        yield jnp.concatenate([lo[:, -128:], hi[:, -128:]], axis=0).astype(BF)


def _conv_phase(q_hbm, k_hbm, v_hbm, sk_ref, h_hbm, sd_ref, w1_hbm, w2_hbm, w3_hbm, w4_hbm,
                l1_ref, l2_ref, l3_ref, l4_ref, q_v, w1_v, w2_v, w3_v, w4_v, y_v,
                k_v, v_v, f_v, kf_s, kv_s, ft_s, a_s, b_s, s1, s2, s3, sem_c, sem_q, sem_w):
    weights = ((w1_hbm, w1_v), (w2_hbm, w2_v), (w3_hbm, w3_v))

    stage = (s1, s2, s3)

    def filter_copy(c):
        return pltpu.make_async_copy(h_hbm.at[pl.ds(c * CB, CB), :], f_v.at[c], sem_c.at[2, c])

    def kv_copies(c):
        cs = pl.ds(c * CB, CB)
        return (pltpu.make_async_copy(k_hbm.at[:, cs], k_v.at[c], sem_c.at[0, c]),
                pltpu.make_async_copy(v_hbm.at[:, cs], v_v.at[c], sem_c.at[1, c]))

    def weight_copies(c):
        return [cp for i, (w_hbm, w_v) in enumerate(weights)
                for cp in _weight_copies(w_hbm, w_v, stage[i].at[c % 2], c, sem_w.at[c * 3 + i])]

    def prep_weights(c):
        for (_, w_v), st in zip(weights, stage):
            yield from _prep_weight(w_v, st.at[c % 2], c)

    def load_filter(c):
        for i in range(S // 128):
            t = f_v[c, :, i * 128:(i + 1) * 128].astype(F32).T
            ft_s[2 * i:2 * i + 2] = t.reshape(2, 8, 8, CB)
            yield t[:RG, :128].astype(BF)

    q_copy = pltpu.make_async_copy(q_hbm, q_v, sem_q.at[0])
    for cp in (filter_copy(0), *kv_copies(0)):
        cp.start()
    for cp in weight_copies(0):
        cp.start()
    kf_s[0:PAD, :] = jnp.zeros((PAD, CB), F32)
    filter_copy(0).wait()
    _run(load_filter(0))

    def conv_block(c, carry):

        @pl.when(c + 1 < NCB)
        def _():
            for cp in (filter_copy(c + 1), *kv_copies(c + 1)):
                cp.start()
            for cp in weight_copies(c + 1):
                cp.start()

        @pl.when(c + 1 == NCB)
        def _():
            q_copy.start()

        for cp in kv_copies(c):
            cp.wait()

        def short_conv():
            kf_s[PAD:PAD + S, :] = k_v[c].astype(F32)
            sk = sk_ref[c]
            rc = 128
            for r in range(S // rc):
                k0 = kf_s[r * rc:PAD + (r + 1) * rc, :]
                k1 = pltpu.roll(k0, 1, 0)
                near = k0 * sk[0:1, :] + k1 * sk[1:2, :]
                far = k0 * sk[2:3, :] + k1 * sk[3:4, :]
                ks = near[PAD:] + far[PAD - 2:PAD - 2 + rc]
                kv = ks * v_v[c, r * rc:(r + 1) * rc, :].astype(F32)
                kv_s[r * 2:(r + 1) * 2] = kv.reshape(2, 8, 8, CB)
                yield kv[:RG, :128].astype(BF)

        def stage1(src, off):
            for j in range(2):
                for g in range(8):
                    tie = yield
                    rhs = src[j * N1:(j + 1) * N1, g].reshape(N1 * 8, CB).astype(BF)
                    out = _pack_groups(_dot(l1_ref[...], _tied(rhs, tie)))
                    for h in range(CB // 128):
                        col = (4 * h + off + j) * 128
                        a_s[:, 8 * g:8 * g + 8, col:col + 128] = out[:, :, h * 128:(h + 1) * 128]

        def stage2():
            def forward(k1, tie):
                out = _dot(l2_ref[k1], _tied(a_s.bitcast(BF)[k1], tie))
                return out

            nxt = forward(0, (yield))
            for k1 in range(N1):
                xf = nxt
                if k1 + 1 < N1:
                    nxt = forward(k1 + 1, (yield))
                xf = xf.reshape(8, 2, 8, 4 * CB)
                zs = []
                for h in range(CB // 128):
                    x0r, x1r, h0r, h1r = (xf[:, 0, :, (4 * h + i) * 128:(4 * h + i + 1) * 128] for i in range(4))
                    x0i, x1i, h0i, h1i = (xf[:, 1, :, (4 * h + i) * 128:(4 * h + i + 1) * 128] for i in range(4))
                    g1r = h1r + h0i
                    g1i = h1i - h0r
                    z0r = x0r * h0r - x0i * h0i
                    z0i = x0r * h0i + x0i * h0r
                    z1r = x0r * g1r - x0i * g1i + (x1r * h0r - x1i * h0i)
                    z1i = x0r * g1i + x0i * g1r + (x1r * h0i + x1i * h0r)
                    zs += [_pack(z0r, z0i), _pack(z1r, z1i)]
                z = pltpu.bitcast(jnp.concatenate(zs, axis=-1).reshape(N2, 2 * CB), BF)
                tie = yield
                b_s[:, 8 * k1:8 * k1 + 8] = _pack_groups(_dot(l3_ref[k1], _tied(z, tie)))

        def stage3():
            sd = sd_ref[c]
            for g in range(8):
                tie = yield
                yv = _dot(l4_ref[...], _tied(b_s.bitcast(BF)[g], tie))
                for j in range(2):
                    yj = jnp.concatenate(
                        [yv[:, (2 * h + j) * 128:(2 * h + j + 1) * 128] for h in range(CB // 128)], axis=1)
                    kvg = kv_s[j * N1:(j + 1) * N1, g]
                    kv_s[j * N1:(j + 1) * N1, g] = yj.reshape(N1, 8, CB) + kvg * sd

        _run(stage1(ft_s, 2), short_conv())
        _run(stage1(kv_s, 0))
        for cp in weight_copies(c):
            cp.wait()
        _run(stage2(), pairs(prep_weights(c)))
        nc = jnp.minimum(c + 1, NCB - 1)

        @pl.when(c + 1 < NCB)
        def _():
            filter_copy(c + 1).wait()

        _run(stage3(), pairs(load_filter(nc)))
        y_v[c] = kv_s[...].reshape(NT, TM, CB).astype(BF)
        return carry

    lax.fori_loop(0, NCB, conv_block, 0)
    q_copy.wait()


def _mlp_phase(w4_hbm, o_hbm, q_v, w1_v, w2_v, w3_v, w4_v, y_v,
               x1_s, xn_s, xp_s, res_s, x2_s, h_s, xa_s, xh_s, xb_s, g_s, o_s, s4, sem_4, sem_o):
    w4_copies = _weight_copies(w4_hbm, w4_v, s4, 0, sem_4)
    for cp in w4_copies:
        cp.start()
    zpad = jnp.zeros((PAD, D), F32)
    for layer in range(2):
        h_s[layer, 0:PAD, :] = zpad
        h_s[layer, PAD + S:PAD + S + PAD, :] = zpad

    def both(ref, g):
        return jnp.concatenate([ref[i * HM + g * RB:i * HM + (g + 1) * RB, :] for i in range(2)], axis=0)

    def put(ref, g, val):
        for i in range(2):
            ref[i * HM + g * RB:i * HM + (g + 1) * RB, :] = val[i * RB:(i + 1) * RB]

    def gate(v, order=None):
        t, slot = v % NT, v % RING
        last = None
        for g in range(HM // RB):
            x = jnp.where(v < NT, both(q_v.at[t], g).astype(F32), both(x2_s.at[t], g))
            x = _after(x, order)
            xl = yield from _ln_steps(x, order)
            y = jnp.concatenate([both(y_v.at[c, t], g) for c in range(NCB)], axis=1).astype(F32)
            x1 = x + xl * y
            put(x1_s.at[slot], g, x1)
            xn = yield from _ln_steps(x1, order)
            put(xn_s.at[slot], g, xn)
            xa = yield from _ln_steps(xn, order)
            last = _store_lhs(xa_s.at[0], g, xa)
            yield last

    def project(v):
        r0 = pl.multiple_of((v % NT) * TM + PAD, 8)
        for n in range(HD // NC):
            cs = yield from _strassen(xa_s.at[v // (32 + n)], w1_v, n)
            for (i, j), c in cs.items():
                h_s[v // NT, pl.ds(r0 + i * HM, HM), j * HD + n * NC:j * HD + (n + 1) * NC] = _gelu(c)

    def shift(v):
        c4 = D // 4

        def fn(r):
            r0 = pl.multiple_of((v % NT) * TM + r, 8)
            parts = []
            for gi, sh in enumerate((1, -1, 2, -2)):
                w = h_s[v // NT, pl.ds(r0, RB + 2 * PAD), gi * c4:(gi + 1) * c4]
                parts.append(w[PAD - sh:PAD - sh + RB])
            return jnp.concatenate(parts, axis=1)
        for g in range(HM // RB):
            yield _store_lhs(xh_s.at[0], g, jnp.concatenate([fn(i * HM + g * RB) for i in range(2)], axis=0))

    def mix(v, order=None):
        for n in range(HD // NC):
            cs = yield from _strassen(xh_s.at[v // (32 + n)], w2_v, n, order)
            for (i, j), c in cs.items():
                rs = slice(i * HM, (i + 1) * HM)
                cols = slice(j * HD + n * NC, j * HD + (n + 1) * NC)
                xp_s[rs, cols] = xn_s[v % RING, rs, cols] + c

    def norm(v, order=None):
        last = None
        for g in range(HM // RB):
            xp = _after(both(xp_s, g), order)
            put(res_s.at[v % 2], g, xp)
            xb = yield from _ln_steps(xp, order)
            last = _store_lhs(xb_s.at[0], g, xb)
            yield last

    def up(u, order):
        for n in range(HF // NC):
            cs = yield from _strassen(xb_s.at[u // (32 + n)], w3_v, n, order)
            g = {ij: _gelu(c) for ij, c in cs.items()}
            for i, t in enumerate(_lhs_terms(g[0, 0], g[0, 1], g[1, 0], g[1, 1])):
                g_s[0, i, :, n * NC:(n + 1) * NC] = t.astype(BF)

    def down(u, order):
        for n in range(HD // NC):
            cs = yield from _strassen(g_s.at[u // (32 + n)], w4_v, n, order)
            for (i, j), c in cs.items():
                rs = slice(i * HM, (i + 1) * HM)
                cols = slice(j * HD + n * NC, j * HD + (n + 1) * NC)
                x2 = x1_s[u % RING, rs, cols] + (res_s[u % 2, rs, cols] + c)
                x2_s[u % NT, rs, cols] = x2
                o_s[u % NT, rs, cols] = x2.astype(BF)

    def out_copy(i):
        return pltpu.make_async_copy(o_s.at[i], o_hbm.at[i], sem_o.at[i])

    def prologue(v, carry):
        _run(gate(v))
        _run(project(v))
        return carry

    lax.fori_loop(0, AHEAD, prologue, 0)
    for cp in w4_copies:
        cp.wait()
    _run(_chain(shift(0), mix(0), norm(0)), _prep_weight(w4_v, s4, 0))

    def main(u, carry):
        nxt = jnp.minimum(u + 1, 2 * NT - 1)
        never = u < 0
        order = [never]
        _run(up(u, order), shift(nxt), every=20, never=never)
        _run(mix(nxt, order))
        _run(down(u, order), _merge(gate(u + AHEAD, order), norm(nxt, order)), every=1, never=never)

        @pl.when(u + AHEAD < 2 * NT)
        def _():
            _run(project(u + AHEAD))

        @pl.when(u >= NT)
        def _():
            out_copy(u - NT).start()

        return carry

    lax.fori_loop(0, 2 * NT, main, 0)
    for i in range(NT):
        out_copy(i).wait()


def _kernel(*refs):
    ins, o_hbm, shared = refs[:14], refs[14], refs[15:]
    pl.run_scoped(
        functools.partial(_conv_phase, *ins, *shared),
        pltpu.VMEM((NCB, S, CB), BF),
        pltpu.VMEM((NCB, S, CB), BF),
        pltpu.VMEM((NCB, CB, S), BF),
        pltpu.VMEM((PAD + S, CB), F32),
        pltpu.VMEM((2 * N1, 8, 8, CB), F32),
        pltpu.VMEM((2 * N1, 8, 8, CB), F32),
        pltpu.VMEM((N1, N2, 4 * CB), U32),
        pltpu.VMEM((8, N1 * 8, 2 * CB), U32),
        *(pltpu.VMEM((2, 2, k // 2 // NCB, n), U32) for k, n in W_HALVES[:3]),
        pltpu.SemaphoreType.DMA((3, NCB)),
        pltpu.SemaphoreType.DMA((1,)),
        pltpu.SemaphoreType.DMA((NCB * 3, 4)),
    )
    lhs = pltpu.VMEM((1, 7, HM, HD), BF)
    pl.run_scoped(
        functools.partial(_mlp_phase, ins[9], o_hbm, *shared),
        pltpu.VMEM((RING, TM, D), F32), pltpu.VMEM((RING, TM, D), F32), pltpu.VMEM((TM, D), F32),
        pltpu.VMEM((2, TM, D), F32), pltpu.VMEM((NT, TM, D), F32),
        pltpu.VMEM((2, S + 2 * PAD, D), F32),
        lhs, lhs, lhs,
        pltpu.VMEM((1, 7, HM, HF), BF),
        pltpu.VMEM((NT, TM, D), BF),
        pltpu.VMEM((2, HF // 2, HD), U32),
        pltpu.SemaphoreType.DMA((4,)),
        pltpu.SemaphoreType.DMA((NT,)),
    )


@jax.jit
def pallas_interleave_layers__ssm_conv_h3__mixer_s_mlp__prompt_kernel(
    A_q, A_k, A_v, A_shift_k, A_ssm_k, A_ssm_D, B_x, B_w1, B_w2, B_w3, B_w4,
):
    del B_x
    l1, l2, l3, l4 = (jnp.asarray(m, dtype=BF) for m in _dft_consts())
    sk = A_shift_k.astype(F32).T.reshape(KS, NCB, CB).transpose(1, 0, 2)
    sd = A_ssm_D.astype(F32).reshape(NCB, 1, CB)
    hbm = pl.BlockSpec(memory_space=pl.ANY)
    vmem = pl.BlockSpec(memory_space=pltpu.VMEM)
    out = pl.pallas_call(
        _kernel,
        out_shape=jax.ShapeDtypeStruct((NT, TM, D), BF),
        in_specs=[hbm, hbm, hbm, vmem, hbm, vmem, hbm, hbm, hbm, hbm, vmem, vmem, vmem, vmem],
        out_specs=hbm,
        scratch_shapes=[
            pltpu.VMEM((NT, TM, D), BF),
            *([pltpu.VMEM((5, k // 2, n), U32), pltpu.VMEM((2, k // 2, n), U32)] for k, n in W_HALVES),
            pltpu.VMEM((NCB, NT, TM, CB), BF),
        ],
        compiler_params=pltpu.CompilerParams(vmem_limit_bytes=120 * 1024 * 1024),
    )(A_q.reshape(NT, TM, D), A_k.reshape(S, D), A_v.reshape(S, D), sk, A_ssm_k, sd,
      B_w1, B_w2, B_w3, B_w4, l1, l2, l3, l4)
    return out.reshape(1, S, D)
```
